```python
import jax
import jax.numpy as jnp

def _softmax(x, axis=-1):
    return jax.nn.softmax(x, axis=axis)
def _gelu(x):
    return jax.nn.gelu(x, approximate=True)
def _silu(x):
    return jax.nn.silu(x)
def _sigmoid(x):
    return jax.nn.sigmoid(x)
def _layernorm(x, axis=-1, eps=1e-5):
    m = jnp.mean(x, axis=axis, keepdims=True)
    v = jnp.var(x, axis=axis, keepdims=True)
    return (x - m) / jnp.sqrt(v + eps)
def _scatter_add(tgt, idx, src, axis=0):
    return tgt.at[idx].add(src)
def _segment_sum(src, seg, n):
    return jax.ops.segment_sum(src, seg, n)
class _Rng:
    def __init__(self, key):
        self._k = key
    def _next(self):
        self._k, sub = jax.random.split(self._k)
        return sub
    def normal(self, shape):
        return jax.random.normal(self._next(), shape, dtype=jnp.bfloat16)
    def randint(self, lo, hi, shape):
        return jax.random.randint(self._next(), shape, lo, hi, dtype=jnp.int32)
    def uniform(self, shape, lo=0.0, hi=1.0):
        return jax.random.uniform(self._next(), shape, jnp.bfloat16, lo, hi)
    def permutation(self, n):
        return jax.random.permutation(self._next(), n)


kernel_name = 'standalone__cross_network_dcn__recsys'

def setup_inputs():
    _rng = _Rng(jax.random.key(int.from_bytes(__import__("os").urandom(4), "little")))
    _w = (lambda a: (lambda t: t.astype(jnp.bfloat16) if jnp.issubdtype(t.dtype, jnp.floating) else t)(jnp.asarray(a)))
    B, F, D, L = 16384, 100, 16, 6
    Din = min(F * D, 1024)
    return {
        "x0": _w((lambda *s: _rng.normal(s) * 0.05)(B, Din)),
        "ws": _w((lambda *s: _rng.normal(s) * 0.05)(L, Din, Din) * (Din ** -0.5)),
        "bs": _w((lambda *s: _rng.normal(s) * 0.05)(L, Din) * 0.01),
    }

def reference(x0, ws, bs):
    x = x0
    L = ws.shape[0]
    for l in range(L):
        proj = jnp.einsum('bd,de->be', x, ws[l]) + bs[l]
        x = x0 * proj + x
    return x
```

```python
import jax, jax.numpy as jnp
from jax import lax
import jax.experimental.pallas as pl
import jax.experimental.pallas.tpu as pltpu

def make(TM, F, SUB=None, NSPLIT0=1, OSPLIT=1, AHEAD=1):
    SUB = SUB or TM
    def f(x0, ws, bs):
        B, D = x0.shape
        L = ws.shape[0]
        n = (B - F) // TM
        assert F + n * TM == B
        f32, bf16 = jnp.float32, jnp.bfloat16

        def layer(xb, x0f, w, b):
            p = jnp.dot(xb, w, preferred_element_type=f32) + b
            return (x0f * p + xb.astype(f32)).astype(bf16)

        def kern(x_hbm, w_hbm, b_hbm, o_hbm, wbuf, bbuf, b32, xf, of, xbuf, obuf, wsem, fsem, xsem, osem):
            def wcopy(l):
                return pltpu.make_async_copy(w_hbm.at[l], wbuf.at[l], wsem.at[l])
            CN = D // NSPLIT0
            def w0copy(j):
                c = pl.ds(j * CN, CN)
                return pltpu.make_async_copy(w_hbm.at[0, :, c], wbuf.at[0, :, c], fsem.at[3 + j])
            def xcopy(i, slot):
                return pltpu.make_async_copy(x_hbm.at[pl.ds(F + i * TM, TM)], xbuf.at[slot], xsem.at[slot])
            OS = TM // OSPLIT
            def ocopy(i, slot, j):
                return pltpu.make_async_copy(obuf.at[slot, pl.ds(j * OS, OS)], o_hbm.at[pl.ds(F + i * TM + j * OS, OS)], osem.at[slot, j])
            xfc = pltpu.make_async_copy(x_hbm.at[pl.ds(0, F)], xf, fsem.at[0])
            bc = pltpu.make_async_copy(b_hbm, bbuf, fsem.at[1])
            ofc = pltpu.make_async_copy(of, o_hbm.at[pl.ds(0, F)], fsem.at[2])
            xfc.start()
            w0copy(0).start()
            bc.start()
            for j in range(1, NSPLIT0):
                w0copy(j).start()
            xfc.wait(); bc.wait()
            b32[...] = bbuf[...].astype(f32)
            for j in range(NSPLIT0):
                w0copy(j).wait()
                if j == NSPLIT0 - 1:
                    for l in range(1, 1 + AHEAD):
                        wcopy(l).start()
                c = slice(j * CN, (j + 1) * CN)
                xc = xf[:, c].astype(f32)
                p = jnp.dot(xf[...], wbuf[0, :, c], preferred_element_type=f32) + b32[0:1, c]
                of[:, c] = (xc * p + xc).astype(bf16)
            def first_layers(l, _):
                wcopy(l).wait()
                @pl.when(l + AHEAD < L)
                def _():
                    wcopy(l + AHEAD).start()
                @pl.when(l + AHEAD == L)
                def _():
                    xcopy(0, 0).start()
                of[...] = layer(of[...], xf[...].astype(f32), wbuf[l], b32[pl.ds(l, 1), :])
                return 0
            lax.fori_loop(1, L, first_layers, 0)
            ofc.start()

            def body(i, _):
                slot = i % 2
                xcopy(i, slot).wait()
                @pl.when(i + 1 < n)
                def _():
                    xcopy(i + 1, 1 - slot).start()
                @pl.when(i >= 2)
                def _():
                    for j in range(OSPLIT):
                        ocopy(i - 2, slot, j).wait()
                for s in range(TM // SUB):
                    rows = pl.ds(s * SUB, SUB)
                    xb = xbuf[slot, rows, :]
                    x0f = xb.astype(f32)
                    for l in range(L):
                        xb = layer(xb, x0f, wbuf[l], b32[l:l + 1, :])
                    obuf[slot, rows, :] = xb
                    for j in range(OSPLIT):
                        if s * SUB < (j + 1) * OS <= (s + 1) * SUB:
                            ocopy(i, slot, j).start()
                return 0
            lax.fori_loop(0, n, body, 0)
            ofc.wait()
            for i in (n - 2, n - 1):
                for j in range(OSPLIT):
                    ocopy(i, i % 2, j).wait()

        anyspec = pl.BlockSpec(memory_space=pl.ANY)
        return pl.pallas_call(
            kern,
            in_specs=[anyspec, anyspec, anyspec],
            out_specs=anyspec,
            out_shape=jax.ShapeDtypeStruct((B, D), x0.dtype),
            scratch_shapes=[
                pltpu.VMEM((L, D, D), bf16), pltpu.VMEM((L, D), bf16), pltpu.VMEM((L, D), f32),
                pltpu.VMEM((F, D), bf16), pltpu.VMEM((F, D), bf16),
                pltpu.VMEM((2, TM, D), bf16), pltpu.VMEM((2, TM, D), bf16),
                pltpu.SemaphoreType.DMA((L,)), pltpu.SemaphoreType.DMA((3 + NSPLIT0,)),
                pltpu.SemaphoreType.DMA((2,)), pltpu.SemaphoreType.DMA((2, OSPLIT)),
            ],
            compiler_params=pltpu.CompilerParams(vmem_limit_bytes=100 * 1024 * 1024),
        )(x0, ws, bs)
    return f


@jax.jit
def pallas_standalone__cross_network_dcn__recsys_kernel(x0, ws, bs):
    return make(512, 512, NSPLIT0=2, AHEAD=2)(x0, ws, bs)
```

```python
import jax
import jax.numpy as jnp
from jax import lax
import jax.experimental.pallas as pl
import jax.experimental.pallas.tpu as pltpu

_TM = 512
_LANE = 128
_K_SLABS = (1, 2, 2, 3)
_SLABS_AHEAD = 3
_W_AHEAD = 2
_OUT_PIECES = 4


def _cross_network(x0, ws, bs, **call_kwargs):
    B, D = x0.shape
    L = ws.shape[0]
    TM = _TM
    n = B // TM - 1
    n_slabs = len(_K_SLABS)
    unit = D // sum(_K_SLABS)
    CN = D // _OUT_PIECES
    assert B % TM == 0 and n >= 2 and L > _W_AHEAD
    assert unit * sum(_K_SLABS) == D and unit % _LANE == 0 and CN % _LANE == 0
    slabs = [slice(sum(_K_SLABS[:j]) * unit, sum(_K_SLABS[:j + 1]) * unit) for j in range(n_slabs)]
    f32 = jnp.float32
    dt = x0.dtype

    def cross(proj, x0f, x):
        return (x0f * proj + x.astype(f32)).astype(dt)

    def kernel(x_hbm, w_hbm, b_hbm, o_hbm,
               wbuf, w0cols, bbuf, b32, xf, of, acc, xbuf, obuf,
               wsem, ssem, fsem, xsem, osem):
        def w_copy(l):
            return pltpu.make_async_copy(w_hbm.at[l], wbuf.at[l], wsem.at[l])

        def slab_copies(j):
            k = slabs[j]
            return (pltpu.make_async_copy(x_hbm.at[pl.ds(0, TM), k], xf.at[:, k], ssem.at[0, j]),
                    pltpu.make_async_copy(w_hbm.at[0, k], wbuf.at[0, k], ssem.at[1, j]))

        def x_copy(i, slot):
            return pltpu.make_async_copy(x_hbm.at[pl.ds((i + 1) * TM, TM)], xbuf.at[slot], xsem.at[slot])

        def o_copy(i, slot, j):
            dst = o_hbm.at[pl.ds((i + 1) * TM, TM), pl.ds(j * CN, CN)]
            return pltpu.make_async_copy(obuf.at[slot, j], dst, osem.at[slot])

        def o_wait(slot):
            pltpu.make_async_copy(obuf.at[slot], obuf.at[slot], osem.at[slot]).wait()

        b_copy = pltpu.make_async_copy(b_hbm, bbuf, fsem.at[0])
        of_copy = pltpu.make_async_copy(of, o_hbm.at[pl.ds(0, TM)], fsem.at[1])

        def first_tile():
            for j in range(_SLABS_AHEAD):
                for c in slab_copies(j):
                    c.start()
                if j == 0:
                    b_copy.start()
            for j in range(n_slabs):
                last = j == n_slabs - 1
                for c in slab_copies(j):
                    c.wait()
                if last:
                    b_copy.wait()
                if j + _SLABS_AHEAD < n_slabs:
                    for c in slab_copies(j + _SLABS_AHEAD):
                        c.start()
                if j == n_slabs - 2:
                    for l in range(1, 1 + _W_AHEAD):
                        w_copy(l).start()
                p = jnp.dot(xf[:, slabs[j]], wbuf[0, slabs[j], :], preferred_element_type=f32)
                if j > 0:
                    p = p + acc[...]
                if not last:
                    acc[...] = p
                else:
                    bias = bbuf[...].astype(f32)
                    b32[...] = bias
                    x = xf[...]
                    of[...] = cross(p + bias[0:1, :], x.astype(f32), x)
                    for t in range(D // _LANE):
                        w0cols[t] = wbuf[0, :, t * _LANE:(t + 1) * _LANE]

            def layer(l, carry):
                @pl.when(l + _W_AHEAD < L)
                def _():
                    w_copy(l + _W_AHEAD).start()

                @pl.when(l + _W_AHEAD == L)
                def _():
                    x_copy(0, 0).start()

                w_copy(l).wait()
                x = of[...]
                p = jnp.dot(x, wbuf[l], preferred_element_type=f32) + b32[pl.ds(l, 1), :]
                of[...] = cross(p, xf[...].astype(f32), x)
                return carry

            lax.fori_loop(1, L, layer, 0)
            of_copy.start()
            x_copy(0, 0).wait()

        def tile(i, carry):
            slot = i % 2

            @pl.when(i + 1 < n)
            def _():
                x_copy(i + 1, 1 - slot).start()

            x = xbuf[slot]
            x0f = x.astype(f32)
            for l in range(L - 1):
                if l == 0:
                    w = jnp.concatenate([w0cols[t] for t in range(D // _LANE)], axis=1)
                else:
                    w = wbuf[l]
                p = jnp.dot(x, w, preferred_element_type=f32) + b32[l:l + 1, :]
                x = cross(p, x0f, x)
            for j in range(_OUT_PIECES):
                c = slice(j * CN, (j + 1) * CN)
                p = jnp.dot(x, wbuf[L - 1, :, c], preferred_element_type=f32) + b32[L - 1:L, c]
                obuf[slot, j] = cross(p, x0f[:, c], x[:, c])
                o_copy(i, slot, j).start()

            @pl.when(i >= 1)
            def _():
                o_wait(1 - slot)

            @pl.when(i + 1 < n)
            def _():
                x_copy(i + 1, 1 - slot).wait()

            return carry

        step = pl.program_id(0)
        half = n // 2
        pl.when(step == 0)(first_tile)
        lax.fori_loop(step * half, half + step * (n - half), tile, 0)

        @pl.when(step == 0)
        def _():
            of_copy.wait()

        @pl.when(step == 1)
        def _():
            o_wait((n - 1) % 2)

    hbm = pl.BlockSpec(memory_space=pl.ANY)
    return pl.pallas_call(
        kernel,
        grid=(2,),
        in_specs=[hbm, hbm, hbm],
        out_specs=hbm,
        out_shape=jax.ShapeDtypeStruct((B, D), dt),
        scratch_shapes=[
            pltpu.VMEM((L, D, D), ws.dtype),
            pltpu.VMEM((D // _LANE, D, _LANE), ws.dtype),
            pltpu.VMEM((L, D), bs.dtype),
            pltpu.VMEM((L, D), f32),
            pltpu.VMEM((TM, D), dt),
            pltpu.VMEM((TM, D), dt),
            pltpu.VMEM((TM, D), f32),
            pltpu.VMEM((2, TM, D), dt),
            pltpu.VMEM((2, _OUT_PIECES, TM, CN), dt),
            pltpu.SemaphoreType.DMA((L,)),
            pltpu.SemaphoreType.DMA((2, n_slabs)),
            pltpu.SemaphoreType.DMA((2,)),
            pltpu.SemaphoreType.DMA((2,)),
            pltpu.SemaphoreType.DMA((2,)),
        ],
        compiler_params=pltpu.CompilerParams(
            dimension_semantics=("arbitrary",),
            vmem_limit_bytes=96 * 1024 * 1024,
        ),
        **call_kwargs,
    )(x0, ws, bs)


@jax.jit
def pallas_standalone__cross_network_dcn__recsys_kernel(
    x0: jax.Array,
    ws: jax.Array,
    bs: jax.Array,
):
    return _cross_network(x0, ws, bs)
```
